```python
import jax
import jax.numpy as jnp

def _softmax(x, axis=-1):
    return jax.nn.softmax(x, axis=axis)
def _gelu(x):
    return jax.nn.gelu(x, approximate=True)
def _silu(x):
    return jax.nn.silu(x)
def _sigmoid(x):
    return jax.nn.sigmoid(x)
def _layernorm(x, axis=-1, eps=1e-5):
    m = jnp.mean(x, axis=axis, keepdims=True)
    v = jnp.var(x, axis=axis, keepdims=True)
    return (x - m) / jnp.sqrt(v + eps)
def _scatter_add(tgt, idx, src, axis=0):
    return tgt.at[idx].add(src)
def _segment_sum(src, seg, n):
    return jax.ops.segment_sum(src, seg, n)
class _Rng:
    def __init__(self, key):
        self._k = key
    def _next(self):
        self._k, sub = jax.random.split(self._k)
        return sub
    def normal(self, shape):
        return jax.random.normal(self._next(), shape, dtype=jnp.bfloat16)
    def randint(self, lo, hi, shape):
        return jax.random.randint(self._next(), shape, lo, hi, dtype=jnp.int32)
    def uniform(self, shape, lo=0.0, hi=1.0):
        return jax.random.uniform(self._next(), shape, jnp.bfloat16, lo, hi)
    def permutation(self, n):
        return jax.random.permutation(self._next(), n)


kernel_name = 'parallel_sum__compressed_kv_cla__moe_arch_mod__prompt'

def setup_inputs():
    _rng = _Rng(jax.random.key(int.from_bytes(__import__("os").urandom(4), "little")))
    _w = (lambda a: (lambda t: t.astype(jnp.bfloat16) if jnp.issubdtype(t.dtype, jnp.floating) else t)(jnp.asarray(a)))
    def _A_setup():
        B, H, Sq, Sk, D, M = 1, 32, 2048, 2048, 128, 640
        Dc = 4 * D
        return {
            "x": _w((lambda *s: _rng.normal(s) * 0.05)(B, Sq, M)),
            "c_kv": _w((lambda *s: _rng.normal(s) * 0.05)(B, Sk, Dc)),
            "w_q": _w((lambda *s: _rng.normal(s) * 0.05)(M, H, D) * (M ** -0.5)),
            "w_uk": _w((lambda *s: _rng.normal(s) * 0.05)(Dc, H, D) * (Dc ** -0.5)),
            "w_uv": _w((lambda *s: _rng.normal(s) * 0.05)(Dc, H, D) * (Dc ** -0.5)),
            "w_o": _w((lambda *s: _rng.normal(s) * 0.05)(H, D, M) * ((H * D) ** -0.5)),
        }
    _A_in = _A_setup()

    def _B_setup():
        B, S, D, F, C = 1, 2048, 640, 1728, 8
        return {
            "x": _w((lambda *s: _rng.normal(s) * 0.05)(B, S, D)),
            "w_r": _w((lambda *s: _rng.normal(s) * 0.05)(D)),
            "w_gate": _w((lambda *s: _rng.normal(s) * 0.05)(D, F)),
            "w_up": _w((lambda *s: _rng.normal(s) * 0.05)(D, F)),
            "w_down": _w((lambda *s: _rng.normal(s) * 0.05)(F, D)),
        }
    _B_in = _B_setup()

    return {
        "A_x": _A_in["x"],
        "A_c_kv": _A_in["c_kv"],
        "A_w_q": _A_in["w_q"],
        "A_w_uk": _A_in["w_uk"],
        "A_w_uv": _A_in["w_uv"],
        "A_w_o": _A_in["w_o"],
        "B_x": _B_in["x"],
        "B_w_r": _B_in["w_r"],
        "B_w_gate": _B_in["w_gate"],
        "B_w_up": _B_in["w_up"],
        "B_w_down": _B_in["w_down"],
    }

def reference(A_x, A_c_kv, A_w_q, A_w_uk, A_w_uv, A_w_o, B_x, B_w_r, B_w_gate, B_w_up, B_w_down):
    def _A_ref(x, c_kv, w_q, w_uk, w_uv, w_o):
        B, Sq, M = x.shape[0], x.shape[1], x.shape[2]
        Sk = c_kv.shape[1]
        H, D = w_q.shape[1], w_q.shape[2]
        q = jnp.einsum("bqm,mhd->bhqd", x, w_q)
        k = jnp.einsum("bkc,chd->bhkd", c_kv, w_uk)
        v = jnp.einsum("bkc,chd->bhkd", c_kv, w_uv)
        scores = jnp.einsum("bhqd,bhkd->bhqk", q, k) * (D ** -0.5)
        off = Sk - Sq
        qi = jnp.arange(Sq)[:, None]
        kj = jnp.arange(Sk)[None, :]
        cmask = kj <= (qi + off)
        scores = jnp.where(cmask[None, None], scores, -1e9)
        p = _softmax(scores, axis=-1)
        ctx = jnp.einsum("bhqk,bhkd->bhqd", p, v)
        return jnp.einsum("bhqd,hdm->bqm", ctx, w_o)

    def _B_ref(x, w_r, w_gate, w_up, w_down):
        B, S, D = x.shape
        C = 8
        r = x @ w_r
        idx = jnp.argsort(-r, axis=-1)[:, :C]
        idx_e = jnp.repeat(idx.reshape(B, C, 1), D, axis=2)
        x_sel = jnp.take_along_axis(x, idx_e, axis=1)
        g = _silu(x_sel @ w_gate)
        u = x_sel @ w_up
        y = (g * u) @ w_down
        r_sel = _sigmoid(jnp.take_along_axis(r, idx, axis=1))
        y = y * r_sel.reshape(B, C, 1)
        b_off = (jnp.arange(B) * S).reshape(B, 1)
        flat_idx = (idx + b_off).reshape(B * C)
        zero = (x * 0.0).reshape(B * S, D)
        upd = _scatter_add(zero, flat_idx, y.reshape(B * C, D), axis=0)
        return x + upd.reshape(B, S, D)

    x = A_x
    xn = _layernorm(x, axis=-1)
    return x + _A_ref(xn, A_c_kv, A_w_q, A_w_uk, A_w_uv, A_w_o) + _B_ref(xn, B_w_r, B_w_gate, B_w_up, B_w_down)
```

```python
import functools
import math
import jax
import jax.numpy as jnp
from jax import lax
import numpy as np
import jax.experimental.pallas as pl
import jax.experimental.pallas.tpu as pltpu

CFG = dict(BQ=256, JO=0, FL=(), FS=(0, 0, 0, 3, 3, 3, 3, 0), PU=1, LA=1)
F32 = jnp.float32
BF16 = jnp.bfloat16
U32 = jnp.uint32
LOG2E = math.log2(math.e)
NT = (((1,), (1,)), ((), ()))
T = 128


def _rb(v):
    return v.astype(BF16).astype(F32)


def _pack(v):
    return pltpu.bitcast(v.astype(BF16), U32)


def _unp(u):
    return pltpu.bitcast(u, BF16)


def _kernel(x_hbm, c_hbm, wq_hbm, wuk_hbm, wuv_hbm, wo_hbm, wr_ref, wg_hbm, wu_hbm, wd_hbm,
            out_hbm,
            x_v, c_v, wq_v, wuk_v, wuv_v, wo_v, wg_v, wu_v, wd_v,
            xn_v, base_v, r_v, q_v, k_v, v_v, ctx_v, o_v, isem, wsem, sems, osems, *, S, M, H, D, DC, F, BQ, C):
    HP = H // 2
    NC = DC // T
    NQ = S // BQ
    NS = BQ // T
    HB = BQ // 2
    c32 = c_hbm.bitcast(U32)
    wo32 = wo_hbm.bitcast(U32)

    def wcopies(p):
        return [pltpu.make_async_copy(h.bitcast(U32).at[:, p, :], v.at[p], wsem.at[p])
                for h, v in ((wuk_hbm, wuk_v), (wuv_hbm, wuv_v), (wq_hbm, wq_v))]

    def incopies(i):
        r0 = pl.multiple_of(i * BQ, BQ)
        h0 = pl.multiple_of(i * HB, HB)
        return ([pltpu.make_async_copy(x_hbm.at[pl.ds(r0, BQ), :], x_v.at[pl.ds(r0, BQ), :], isem.at[i])]
                + [pltpu.make_async_copy(c32.at[pl.ds(h0, HB), t * T:(t + 1) * T], c_v.at[t, pl.ds(h0, HB), :], isem.at[i])
                   for t in range(NC)])

    late = [pltpu.make_async_copy(wo32.at[:, t * T:(t + 1) * T], wo_v.at[t], sems.at[t]) for t in range(M // T)]
    late += [pltpu.make_async_copy(a, b, sems.at[M // T + n])
             for n, (a, b) in enumerate(((wg_hbm, wg_v), (wu_hbm, wu_v), (wd_hbm, wd_v)))]

    for c in incopies(NQ - 1) + wcopies(0) + incopies(NQ - 2):
        c.start()

    qscale = (D ** -0.5) * LOG2E
    NEG = -1e9 * LOG2E

    def whead(buf, h):
        u = buf[h // 2] << (16 * (1 - h % 2)).astype(U32)
        return pltpu.bitcast(u & jnp.uint32(0xFFFF0000), F32).astype(BF16)

    def kv_job(h0, wkv):
        lhs = jnp.concatenate([_unp(c_v[t, pl.ds(h0, HB), :]) for t in range(NC)], axis=1)
        kk = jnp.dot(lhs, wkv, preferred_element_type=F32)
        k_v[pl.ds(h0, HB), :] = _pack(kk[:, :D])
        v_v[pl.ds(h0, HB), :] = _pack(kk[:, D:])

    def q_job(h0, wq, xn=None):
        xn = _unp(xn_v[pl.ds(h0, HB), :]) if xn is None else xn
        q_v[pl.ds(h0, HB), :] = _pack(jnp.dot(xn, wq, preferred_element_type=F32) * qscale)

    def weights(h):
        return jnp.concatenate([whead(wuk_v, h), whead(wuv_v, h)], axis=1), whead(wq_v, h)

    wr = wr_ref[...].astype(F32).reshape(1, M)
    eps = float(np.float32(1e-5).astype(jnp.bfloat16))
    r_v[...] = jnp.zeros(r_v.shape, F32)
    for c in wcopies(0):
        c.wait()

    def ln_body(n, _):
        i = NQ - 1 - n

        @pl.when(i >= 2)
        def _():
            for c in incopies(i - 2):
                c.start()
        for c in incopies(i):
            c.wait()
        r0 = pl.multiple_of(i * BQ, BQ)
        h0 = pl.multiple_of(i * HB, HB)
        wkv, wq = weights(jnp.int32(0))
        kv_job(h0, wkv)
        xf = x_v[pl.ds(r0, BQ), :].astype(F32)
        mean = jnp.sum(xf, axis=1, keepdims=True) * (1.0 / M)
        cen = xf - mean
        var = jnp.sum(cen * cen, axis=1, keepdims=True) * (1.0 / M)
        d = _rb(xf - _rb(mean))
        sd = _rb(jnp.sqrt(_rb(_rb(var) + eps)))
        xn = (d * (1.0 / sd)).astype(BF16)
        xn_v[pl.ds(h0, HB), :] = pltpu.bitcast(xn, U32)
        q_job(h0, wq, xn)
        xnf = xn.astype(F32)
        base_v[pl.ds(r0, BQ), :] = xf + xnf
        r = _rb(jnp.sum(xnf * wr, axis=1, keepdims=True))
        g0 = (r0 // 8) % 128
        grp = lax.broadcasted_iota(jnp.int32, (BQ, 128), 0) // 8
        lane = lax.broadcasted_iota(jnp.int32, (BQ, 128), 1) - g0
        rr = r_v[r0 // 1024]
        for g in range(BQ // 8):
            rr = jnp.where(lane[:8] == g, r[8 * g:8 * g + 8], rr)
        r_v[r0 // 1024] = rr
        return 0
    with jax.named_scope('ln'):
        lax.fori_loop(0, NQ, ln_body, 0, unroll=CFG["PU"])
    for c in wcopies(1) + late:
        c.start()

    def allred(a, red):
        a = red(a, axis=0)
        return red(red(a, axis=0, keepdims=True), axis=1, keepdims=True)

    def route():
        rv = r_v[...]
        tok = (lax.broadcasted_iota(jnp.int32, rv.shape, 0) * 1024 + lax.broadcasted_iota(jnp.int32, rv.shape, 2) * 8
               + lax.broadcasted_iota(jnp.int32, rv.shape, 1)).astype(F32)
        isn = rv != rv
        key = jnp.where(isn, -jnp.inf, rv)
        pri = jnp.where(isn, tok + S, tok)
        BIG = float(4 * S)
        idxs, rows, scs = [], [], []
        for c in range(C):
            mx = allred(key, jnp.max)
            pi = allred(jnp.where(key == mx, pri, BIG), jnp.min)
            took = pri == pi
            key = jnp.where(took, -jnp.inf, key)
            pri = jnp.where(took, BIG, pri)
            scs.append(jnp.broadcast_to(jnp.where(pi >= S, jnp.nan, mx), (1, M)))
            ii = jnp.clip(pi.astype(jnp.int32)[0, 0] % S, 0, S - 1)
            idxs.append(ii)
            slab = _unp(xn_v[pl.ds(pl.multiple_of((ii // 16) * 8, 8), 8), :]).astype(F32)
            rows.append(jnp.sum(jnp.where(lax.broadcasted_iota(jnp.int32, slab.shape, 0) == ii % 16, slab, 0.0), axis=0, keepdims=True))
        return idxs, jnp.concatenate(rows, axis=0).astype(BF16), jnp.concatenate(scs, axis=0)

    def ffn_jobs(idxs, xs, sc):
        FC = 512
        cuts = list(range(0, F, FC)) + [F]
        st = {}

        def gate(a, b):
            st["g"] = _rb(lax.dot_general(xs, wg_v[a:b, :], NT, preferred_element_type=F32))

        def up(a, b):
            u = _rb(lax.dot_general(xs, wu_v[a:b, :], NT, preferred_element_type=F32))
            g = st["g"]
            st["h"] = (_rb(g * jax.nn.sigmoid(g)) * u).astype(BF16)

        def down(a, b):
            y = jnp.dot(st["h"], wd_v[a:b, :], preferred_element_type=F32)
            st["y"] = y if "y" not in st else st["y"] + y
            if b == F:
                y = _rb(st["y"]) * _rb(jax.nn.sigmoid(sc))
                for c in range(C):
                    base_v[pl.ds(idxs[c], 1), :] += y[c:c + 1, :]
        return [functools.partial(f, a, b) for a, b in zip(cuts[:-1], cuts[1:]) for f in (gate, up, down)]

    def rows(ref, a, b):
        return _unp(ref[a // 2:b // 2, :])

    def qk(i):
        lo = i * BQ
        out = []
        for t in range(NS):
            k0 = 0 if t == 0 else lo + t * T
            k1 = lo + (t + 1) * T
            out.append(lax.dot_general(rows(q_v, lo + t * T, lo + BQ), rows(k_v, k0, k1), NT, preferred_element_type=F32))
        return out

    def fold(a, op):
        r = a[:, :T]
        for c in range(1, a.shape[1] // T):
            r = op(r, a[:, c * T:(c + 1) * T])
        return r

    def comb(xs, op):
        out = []
        for r in range(NS):
            o = xs[0][r * T:(r + 1) * T]
            for t in range(1, r + 1):
                o = op(o, xs[t][(r - t) * T:(r - t + 1) * T])
            out.append(o)
        return jnp.concatenate(out, axis=0) if NS > 1 else out[0]

    def pv(h, i, ss):
        tri = lax.broadcasted_iota(jnp.int32, (T, T), 1) <= lax.broadcasted_iota(jnp.int32, (T, T), 0)
        ms = []
        for t in range(NS):
            a = ss[t]
            d = jnp.where(tri, a[:T, -T:], NEG)
            if a.shape[0] > T:
                d = jnp.concatenate([d, a[T:, -T:]], axis=0)
            if a.shape[1] > T:
                d = jnp.concatenate([a[:, :-T], d], axis=1)
            ms.append(d)
        m = jnp.max(comb([fold(a, jnp.maximum) for a in ms], jnp.maximum), axis=1, keepdims=True)
        ps = [jnp.exp2(ms[t] - m[t * T:]) for t in range(NS)]
        l = jnp.sum(comb([fold(p, jnp.add) for p in ps], jnp.add), axis=1, keepdims=True)
        lo = i * BQ
        os_ = []
        for t in range(NS):
            k0 = 0 if t == 0 else lo + t * T
            k1 = lo + (t + 1) * T
            os_.append(jnp.dot(ps[t].astype(BF16), rows(v_v, k0, k1), preferred_element_type=F32))
        r = pl.reciprocal(l, approx=True)
        r = r * (2.0 - l * r)
        ctx_v[h, lo // 2:(lo + BQ) // 2, :] = _pack(comb(os_, jnp.add) * r)

    def head_body(h, _):
        @pl.when(h % 2 == 1)
        def _():
            p = (h + 1) // 2
            for c in wcopies(p):
                c.wait()

            @pl.when(p + 1 < HP)
            def _():
                for c in wcopies(p + 1):
                    c.start()
        wkv, wq = weights(h + 1)
        for i in reversed(range(NQ)):
            ss = qk(i)
            if CFG["JO"] == 0:
                q_job(i * HB, wq)
                if i + 1 < NQ:
                    kv_job((i + 1) * HB, wkv)
            elif CFG["JO"] == 1:
                if i + 1 < NQ:
                    kv_job((i + 1) * HB, wkv)
                q_job(i * HB, wq)
            elif CFG["JO"] == 2:
                if i + 1 < NQ:
                    kv_job((i + 1) * HB, wkv)
                if i > 0:
                    q_job(i * HB, wq)
            pv(h, i, ss)
        if CFG["JO"] == 2:
            q_job(0, wq)
        kv_job(0, wkv)
        return 0
    with jax.named_scope('heads'):
        lax.fori_loop(0, H - 1, head_body, 0)

    for c in late:
        c.wait()
    with jax.named_scope('last'):
        jobs = ffn_jobs(*route())
        sq = {}
        for n in range(NQ + CFG["LA"]):
            if n < NQ:
                sq[n] = qk(NQ - 1 - n)
                for _ in range(CFG["FS"][n]):
                    jobs.pop(0)()
            if n >= CFG["LA"]:
                pv(H - 1, NQ - 1 - (n - CFG["LA"]), sq.pop(n - CFG["LA"]))
        for jb in jobs:
            jb()

    OC = 256

    def ocopy(r0, t):
        return pltpu.make_async_copy(o_v.at[pl.ds(r0, OC), :], out_hbm.at[pl.ds(r0, OC), :], osems.at[t])

    def out_body(t, _):
        r0 = pl.multiple_of(t * OC, OC)
        h0 = pl.multiple_of(t * (OC // 2), OC // 2)
        lhs = jnp.concatenate([_unp(ctx_v[h, pl.ds(h0, OC // 2), :]) for h in range(H)], axis=1)
        wo = jnp.concatenate([_unp(wo_v[n]) for n in range(M // T)], axis=1)
        acc = jnp.dot(lhs, wo, preferred_element_type=F32)
        o_v[pl.ds(r0, OC), :] = (base_v[pl.ds(r0, OC), :] + acc).astype(BF16)
        ocopy(r0, t).start()
        return 0
    with jax.named_scope('oproj'):
        lax.fori_loop(0, S // OC, out_body, 0)
    for t in range(S // OC):
        ocopy(t * OC, t).wait()


@jax.jit
def pallas_parallel_sum__compressed_kv_cla__moe_arch_mod__prompt_kernel(A_x, A_c_kv, A_w_q, A_w_uk, A_w_uv, A_w_o, B_x, B_w_r, B_w_gate, B_w_up, B_w_down):
    del B_x
    B, S, M = A_x.shape
    DC = A_c_kv.shape[2]
    H, D = A_w_q.shape[1], A_w_q.shape[2]
    F = B_w_gate.shape[1]
    hbm = pl.BlockSpec(memory_space=pltpu.HBM)
    V = pltpu.VMEM
    DMA = pltpu.SemaphoreType.DMA
    out = pl.pallas_call(
        functools.partial(_kernel, S=S, M=M, H=H, D=D, DC=DC, F=F, BQ=CFG['BQ'], C=8),
        out_shape=jax.ShapeDtypeStruct((S, M), BF16),
        in_specs=[hbm] * 6 + [pl.BlockSpec(memory_space=pltpu.VMEM)] + [hbm] * 3,
        out_specs=hbm,
        scratch_shapes=[
            V((S, M), BF16), V((DC // T, S // 2, T), U32),
            V((H // 2, M, D), U32), V((H // 2, DC, D), U32), V((H // 2, DC, D), U32),
            V((M // T, H * D // 2, T), U32), V((F, M), BF16), V((F, M), BF16), V((F, M), BF16),
            V((S // 2, M), U32), V((S, M), F32), V((S // 1024, 8, 128), F32),
            *[V((S // 2, D), U32)] * 3,
            V((H, S // 2, D), U32), V((S, M), BF16),
            DMA((S // CFG['BQ'],)), DMA((H // 2,)), DMA((8,)), DMA((8,)),
        ],
        compiler_params=pltpu.CompilerParams(vmem_limit_bytes=110 * 1024 * 1024, flags={k: True for k in CFG['FL']} or None),
        name="mla_mod",
    )(A_x.reshape(S, M), A_c_kv.reshape(S, DC), A_w_q, A_w_uk, A_w_uv, A_w_o.reshape(H * D, M), B_w_r, B_w_gate.T, B_w_up.T, B_w_down)
    return out.reshape(B, S, M)
```

```python
import functools
import math

import jax
import jax.experimental.pallas as pl
import jax.experimental.pallas.tpu as pltpu
import jax.numpy as jnp
import numpy as np
from jax import lax

F32 = jnp.float32
BF16 = jnp.bfloat16
U32 = jnp.uint32
LOG2E = math.log2(math.e)
NT = (((1,), (1,)), ((), ()))
T = 128
BQ = 256
HB = BQ // 2
CAPACITY = 8
JOBS_PER_BLOCK = (1, 1, 1, 1, 1, 3, 3, 4)


def _rb(v):
    return v.astype(BF16).astype(F32)


def _pack(v):
    return pltpu.bitcast(v.astype(BF16), U32)


def _unp(u):
    return pltpu.bitcast(u, BF16)


def _rows(ref, a, b):
    return _unp(ref[a // 2:b // 2, :])


def _fold(a, op):
    r = a[:, :T]
    for c in range(1, a.shape[1] // T):
        r = op(r, a[:, c * T:(c + 1) * T])
    return r


def _stairs(xs, op):
    out = []
    for r in range(len(xs)):
        o = xs[0][r * T:(r + 1) * T]
        for t in range(1, r + 1):
            o = op(o, xs[t][(r - t) * T:(r - t + 1) * T])
        out.append(o)
    return jnp.concatenate(out, axis=0)


def _pieces(i):
    lo = i * BQ
    return [(lo + t * T, lo + t * T if t else 0, lo + (t + 1) * T) for t in range(BQ // T)]


def _mm(lhs, ref, k0, k1, nt, tick):
    if tick is None:
        if nt:
            return lax.dot_general(lhs, _rows(ref, k0, k1), NT, preferred_element_type=F32)
        return jnp.dot(lhs, _rows(ref, k0, k1), preferred_element_type=F32)
    cuts = list(range(k1, k0, -4 * T))[::-1]
    outs = []
    for a, b in zip([k0] + cuts[:-1], cuts):
        outs.append(_mm(lhs if nt else lhs[:, a - k0:b - k0], ref, a, b, nt, None))
        if (b - a) * lhs.shape[0] >= 2 * T * BQ:
            tick()
    return jnp.concatenate(outs, axis=1) if nt else functools.reduce(jnp.add, outs)


def _scores(i, q_ref, k_ref, tick=None):
    return [_mm(_rows(q_ref, r0, (i + 1) * BQ), k_ref, k0, k1, True, tick) for r0, k0, k1 in _pieces(i)]


def _context(i, ss, v_ref, tick=None):
    tri = lax.broadcasted_iota(jnp.int32, (T, T), 1) <= lax.broadcasted_iota(jnp.int32, (T, T), 0)
    ms = []
    for a in ss:
        d = jnp.where(tri, a[:T, -T:], -1e9 * LOG2E)
        if a.shape[0] > T:
            d = jnp.concatenate([d, a[T:, -T:]], axis=0)
        if a.shape[1] > T:
            d = jnp.concatenate([a[:, :-T], d], axis=1)
        ms.append(d)
    m = jnp.max(_stairs([_fold(a, jnp.maximum) for a in ms], jnp.maximum), axis=1, keepdims=True)
    ps = [jnp.exp2(a - m[t * T:]) for t, a in enumerate(ms)]
    l = jnp.sum(_stairs([_fold(p, jnp.add) for p in ps], jnp.add), axis=1, keepdims=True)
    os_ = [_mm(p.astype(BF16), v_ref, k0, k1, False, tick) for p, (_, k0, k1) in zip(ps, _pieces(i))]
    r = pl.reciprocal(l, approx=True)
    r = r * (2.0 - l * r)
    return _pack(_stairs(os_, jnp.add) * r)


def _kernel(x_hbm, c_hbm, wq_hbm, wuk_hbm, wuv_hbm, wo_hbm, wr_hbm, wg_hbm, wu_hbm, wd_hbm, out_hbm,
            x_v, cb_v, c_v, wq_v, wuk_v, wuv_v, wo_v, wg_v, wu_v, wd_v, xn_v, wr_v, r_v,
            q_v, k_v, v_v, q1_v, k1_v, v1_v, ctx_v, o_v, xsem, csem, wsem, sems, osems):
    S, M = x_v.shape
    H, _, D = ctx_v.shape
    F = wd_v.shape[0]
    NQ = S // BQ

    def wcopies(p):
        return [pltpu.make_async_copy(h.bitcast(U32).at[:, p, :], v.at[p], wsem.at[p])
                for h, v in ((wuk_hbm, wuk_v), (wuv_hbm, wuv_v), (wq_hbm, wq_v))]

    def incopies(i):
        at = pl.ds(pl.multiple_of(i * BQ, BQ), BQ)
        return [pltpu.make_async_copy(x_hbm.at[at, :], x_v.at[at, :], xsem.at[i]),
                pltpu.make_async_copy(c_hbm.at[at, :], cb_v.at[at, :], csem.at[i])]

    def ocopy(i):
        at = pl.ds(pl.multiple_of(i * BQ, BQ), BQ)
        return pltpu.make_async_copy(o_v.at[at, :], out_hbm.at[at, :], osems.at[i])

    late = [(wo_hbm.bitcast(U32).at[:, t * T:(t + 1) * T], wo_v.at[t]) for t in range(M // T)]
    late += [(wg_hbm, wg_v), (wu_hbm, wu_v), (wd_hbm, wd_v)]
    late = [pltpu.make_async_copy(a, b, sems.at[n]) for n, (a, b) in enumerate(late)]
    first = wcopies(0) + [pltpu.make_async_copy(wr_hbm, wr_v, sems.at[len(late)])]
    for c in first + incopies(NQ - 1) + incopies(NQ - 2):
        c.start()

    def whead(buf, h):
        u = buf[h // 2] << (16 * (1 - h % 2)).astype(U32)
        return pltpu.bitcast(u & jnp.uint32(0xFFFF0000), F32).astype(BF16)

    def weights(h):
        return jnp.concatenate([whead(wuk_v, h), whead(wuv_v, h)], axis=1), whead(wq_v, h)

    def project(lhs, w, h0, refs, scale=None):
        res = jnp.dot(lhs, w, preferred_element_type=F32)
        if scale is not None:
            res = res * scale
        for n, ref in enumerate(refs):
            ref[pl.ds(h0, HB), :] = _pack(res[:, n * D:(n + 1) * D])

    qscale = (D ** -0.5) * LOG2E

    eps = float(np.float32(1e-5).astype(BF16))
    r_v[...] = jnp.zeros(r_v.shape, F32)
    for c in first:
        c.wait()
    wr = wr_v[...].astype(F32).reshape(1, M)
    wkv0, wq0 = [jnp.concatenate(w, axis=1) for w in zip(weights(jnp.int32(0)), weights(jnp.int32(1)))]

    def ln_body(n, _):
        i = NQ - 1 - n
        for c in incopies(i):
            c.wait()

        @pl.when(i >= 2)
        def _():
            for c in incopies(i - 2):
                c.start()

        @pl.when(i == 1)
        def _():
            for c in wcopies(1):
                c.start()

        r0 = pl.multiple_of(i * BQ, BQ)
        h0 = pl.multiple_of(i * HB, HB)
        cu = pltpu.bitcast(cb_v[pl.ds(r0, BQ), :], U32)
        c_v[pl.ds(h0, HB), :] = cu
        project(_unp(cu), wkv0, h0, (k_v, v_v, k1_v, v1_v))
        xf = x_v[pl.ds(r0, BQ), :].astype(F32)
        mean = jnp.sum(xf, axis=1, keepdims=True) * (1.0 / M)
        cen = xf - mean
        var = jnp.sum(cen * cen, axis=1, keepdims=True) * (1.0 / M)
        sd = _rb(jnp.sqrt(_rb(_rb(var) + eps)))
        xn = (_rb(xf - _rb(mean)) * (1.0 / sd)).astype(BF16)
        xn_v[pl.ds(h0, HB), :] = pltpu.bitcast(xn, U32)
        project(xn, wq0, h0, (q_v, q1_v), qscale)
        r = jnp.sum(xn.astype(F32) * wr, axis=1, keepdims=True)
        lane = lax.broadcasted_iota(jnp.int32, (8, T), 1) - (r0 // 8) % T
        rr = r_v[r0 // (8 * T)]
        for g in range(BQ // 8):
            rr = jnp.where(lane == g, r[8 * g:8 * g + 8], rr)
        r_v[r0 // (8 * T)] = rr
        return 0

    lax.fori_loop(0, NQ, ln_body, 0)

    def head_body(n, _):
        @pl.when(n % 2 == 0)
        def _():
            for c in wcopies(n // 2 + 1):
                c.wait()

            @pl.when(n // 2 + 2 < H // 2)
            def _():
                for c in wcopies(n // 2 + 2):
                    c.start()

            @pl.when(n == 0)
            def _():
                for c in late:
                    c.start()

        h = n + jnp.minimum(n, 1)
        wkv, wq = weights(n + 2)
        todo = [(kv, i) for i in reversed(range(NQ)) for kv in (0, 1)]

        def job(cur):
            kv, i = todo.pop(0)
            assert cur <= i - kv
            if kv:
                project(_rows(c_v, i * BQ, (i + 1) * BQ), wkv, i * HB, (k_v, v_v))
            else:
                project(_rows(xn_v, i * BQ, (i + 1) * BQ), wq, i * HB, (q_v,), qscale)

        for i in reversed(range(NQ)):
            ss = _scores(i, q_v, k_v)
            for _ in range(JOBS_PER_BLOCK[NQ - 1 - i]):
                job(i)
            ctx_v[h, i * HB:(i + 1) * HB, :] = _context(i, ss, v_v)
        while todo:
            job(-1)
        return 0

    lax.fori_loop(0, H - 2, head_body, 0)
    for c in late:
        c.wait()

    def allred(a, red):
        return red(red(red(a, axis=0), axis=0, keepdims=True), axis=1, keepdims=True)

    rv = _rb(r_v[...])
    io = lambda k: lax.broadcasted_iota(jnp.int32, rv.shape, k)
    tok = (io(0) * (8 * T) + io(2) * 8 + io(1)).astype(F32)
    isnan = rv != rv
    key = jnp.where(isnan, -jnp.inf, rv)
    pri = jnp.where(isnan, tok + S, tok)
    taken = float(4 * S)

    def slab(idx):
        at = pl.ds(pl.multiple_of((idx // 16) * 8, 8), 8)
        val = _unp(xn_v[at, :]).astype(F32)
        return at, val, lax.broadcasted_iota(jnp.int32, val.shape, 0) == idx % 16

    idxs, xsel, rsel = [], [], []
    for _ in range(CAPACITY):
        mx = allred(key, jnp.max)
        pi = allred(jnp.where(key == mx, pri, taken), jnp.min)
        hit = pri == pi
        key = jnp.where(hit, -jnp.inf, key)
        pri = jnp.where(hit, taken, pri)
        rsel.append(jnp.broadcast_to(jnp.where(pi >= S, jnp.nan, mx), (1, M)))
        idxs.append(jnp.clip(pi.astype(jnp.int32)[0, 0] % S, 0, S - 1))
        _, val, row = slab(idxs[-1])
        xsel.append(jnp.sum(jnp.where(row, val, 0.0), axis=0, keepdims=True))
    xsel = jnp.concatenate(xsel, axis=0).astype(BF16)
    rsel = jnp.concatenate(rsel, axis=0)

    st = {}

    def add(k, val):
        st[k] = st[k] + val if k in st else val

    def up(k, w_v, a, b, k0, k1):
        add(k, lax.dot_general(xsel[:, k0:k1], w_v[a:b, k0:k1], NT, preferred_element_type=F32))

    def down(a, b, n0, n1):
        if ("h", a) not in st:
            g = _rb(st["g", a])
            st["h", a] = (_rb(g * jax.nn.sigmoid(g)) * _rb(st["u", a])).astype(BF16)
        y = jnp.dot(st["h", a], wd_v[a:b, n0:n1], preferred_element_type=F32)
        for n in range(n0, n1, T):
            add(("y", n), y[:, n - n0:n - n0 + T])

    def scatter():
        y = jnp.concatenate([st["y", n] for n in range(0, M, T)], axis=1)
        y = _rb(_rb(y) * _rb(jax.nn.sigmoid(rsel)))
        for c, idx in enumerate(idxs):
            at, val, row = slab(idx)
            xn_v[at, :] = _pack(jnp.where(row, val + y[c:c + 1, :], val))

    ffn, downs = [], []
    for a in range(0, F, 4 * T):
        b = min(a + 4 * T, F)
        w = T * (4 // pl.cdiv(b - a, T))
        ks = [(k, min(k + w, M)) for k in range(0, M, w)]
        ffn += [functools.partial(up, ("g", a), wg_v, a, b, *k) for k in ks] + downs
        ffn += [functools.partial(up, ("u", a), wu_v, a, b, *k) for k in ks]
        downs = [functools.partial(down, a, b, *k) for k in ks]
    ffn += downs + [scatter]

    def tick():
        if ffn:
            ffn.pop(0)()

    work = [(i, b) for i in reversed(range(NQ)) for b in ((H - 1, q_v, k_v, v_v), (1, q1_v, k1_v, v1_v))]
    prev = None
    for n, cur in enumerate(work + [None]):
        tk = tick if n >= 4 else None
        ss = _scores(cur[0], cur[1][1], cur[1][2], tk) if cur else None
        if prev:
            (i, b), ps = prev
            ctx_v[b[0], i * HB:(i + 1) * HB, :] = _context(i, ps, b[3], tk)
        prev = (cur, ss)

    def ctx_rows(h0, ha, hb):
        return jnp.concatenate([_unp(ctx_v[h, pl.ds(h0, HB), :]) for h in range(ha, hb)], axis=1)

    def finish(i, attn):
        r0 = pl.multiple_of(i * BQ, BQ)
        h0 = pl.multiple_of(i * HB, HB)
        res = (x_v[pl.ds(r0, BQ), :].astype(F32) + attn) + _unp(xn_v[pl.ds(h0, HB), :]).astype(F32)
        o_v[pl.ds(r0, BQ), :] = res.astype(BF16)
        ocopy(i).start()

    cols = []
    for n in range(M // T):
        parts = []
        for h in range(0, H, 4):
            parts.append(jnp.dot(ctx_rows((NQ - 1) * HB, h, h + 4), _rows(wo_v.at[n], h * D, (h + 4) * D),
                                 preferred_element_type=F32))
            tick()
        cols.append(functools.reduce(jnp.add, parts))
    while ffn:
        tick()
    finish(NQ - 1, jnp.concatenate(cols, axis=1))

    def out_body(i, _):
        wo = jnp.concatenate([_unp(wo_v[n]) for n in range(M // T)], axis=1)
        finish(i, jnp.dot(ctx_rows(pl.multiple_of(i * HB, HB), 0, H), wo, preferred_element_type=F32))
        return 0

    lax.fori_loop(0, NQ - 1, out_body, 0)
    for i in range(NQ):
        ocopy(i).wait()


@jax.jit
def pallas_parallel_sum__compressed_kv_cla__moe_arch_mod__prompt_kernel(
    A_x: jax.Array,
    A_c_kv: jax.Array,
    A_w_q: jax.Array,
    A_w_uk: jax.Array,
    A_w_uv: jax.Array,
    A_w_o: jax.Array,
    B_x: jax.Array,
    B_w_r: jax.Array,
    B_w_gate: jax.Array,
    B_w_up: jax.Array,
    B_w_down: jax.Array,
):
    del B_x
    B, S, M = A_x.shape
    DC = A_c_kv.shape[2]
    _, H, D = A_w_q.shape
    F = B_w_gate.shape[1]
    assert B == 1 and A_c_kv.shape[1] == S and D == T and S // BQ == len(JOBS_PER_BLOCK)
    hbm = pl.BlockSpec(memory_space=pltpu.HBM)
    V = pltpu.VMEM
    DMA = pltpu.SemaphoreType.DMA
    out = pl.pallas_call(
        _kernel,
        out_shape=jax.ShapeDtypeStruct((S, M), BF16),
        in_specs=[hbm] * 10,
        out_specs=hbm,
        scratch_shapes=[
            V((S, M), BF16), V((S, DC), BF16), V((S // 2, DC), U32),
            V((H // 2, M, D), U32), V((H // 2, DC, D), U32), V((H // 2, DC, D), U32),
            V((M // T, H * D // 2, T), U32), V((F, M), BF16), V((F, M), BF16), V((F, M), BF16),
            V((S // 2, M), U32), V((M,), BF16), V((S // (8 * T), 8, T), F32),
            *[V((S // 2, D), U32)] * 6,
            V((H, S // 2, D), U32), V((S, M), BF16),
            DMA((S // BQ,)), DMA((S // BQ,)), DMA((H // 2,)), DMA((M // T + 4,)), DMA((S // BQ,)),
        ],
        compiler_params=pltpu.CompilerParams(vmem_limit_bytes=110 * 1024 * 1024),
        name="mla_mod",
    )(A_x.reshape(S, M), A_c_kv.reshape(S, DC), A_w_q, A_w_uk, A_w_uv, A_w_o.reshape(H * D, M),
      B_w_r, B_w_gate.T, B_w_up.T, B_w_down)
    return out.reshape(B, S, M)
```
